```python
import os as _os
_os.environ.setdefault("JAX_PLATFORMS", "cpu")
import jax
import jax.numpy as jnp

def _softmax(x, axis=-1):
    return jax.nn.softmax(x, axis=axis)
def _gelu(x):
    return jax.nn.gelu(x, approximate=True)
def _silu(x):
    return jax.nn.silu(x)
def _sigmoid(x):
    return jax.nn.sigmoid(x)
def _layernorm(x, axis=-1, eps=1e-5):
    m = jnp.mean(x, axis=axis, keepdims=True)
    v = jnp.var(x, axis=axis, keepdims=True)
    return (x - m) / jnp.sqrt(v + eps)
def _scatter_add(tgt, idx, src, axis=0):
    return tgt.at[idx].add(src)
def _segment_sum(src, seg, n):
    return jax.ops.segment_sum(src, seg, n)
class _Rng:
    def __init__(self, key):
        self._k = key
    def _next(self):
        self._k, sub = jax.random.split(self._k)
        return sub
    def normal(self, shape):
        return jax.random.normal(self._next(), shape, dtype=jnp.bfloat16)
    def randint(self, lo, hi, shape):
        return jax.random.randint(self._next(), shape, lo, hi, dtype=jnp.int32)
    def uniform(self, shape, lo=0.0, hi=1.0):
        return jax.random.uniform(self._next(), shape, jnp.bfloat16, lo, hi)
    def permutation(self, n):
        return jax.random.permutation(self._next(), n)


kernel_name = 'gated_mix__compressed_kv_cla__ssm_conv_h3__prompt'

def setup_inputs():
    _rng = _Rng(jax.random.key(int.from_bytes(__import__("os").urandom(4), "little")))
    _w = (lambda a: (lambda t: t.astype(jnp.bfloat16) if jnp.issubdtype(t.dtype, jnp.floating) else t)(jnp.asarray(a)))
    def _A_setup():
        B, H, Sq, Sk, D, M = 1, 32, 2048, 2048, 128, 1024
        Dc = 4 * D
        return {
            "x": _w((lambda *s: _rng.normal(s) * 0.05)(B, Sq, M)),
            "c_kv": _w((lambda *s: _rng.normal(s) * 0.8)(B, Sk, Dc)),
            "w_q": _w((lambda *s: _rng.normal(s) * 3.2)(M, H, D) * (M ** -0.5)),
            "w_uk": _w((lambda *s: _rng.normal(s) * 3.2)(Dc, H, D) * (Dc ** -0.5)),
            "w_uv": _w((lambda *s: _rng.normal(s) * 0.8)(Dc, H, D) * (Dc ** -0.5)),
            "w_o": _w((lambda *s: _rng.normal(s) * 0.8)(H, D, M) * ((H * D) ** -0.5)),
        }
    _A_in = _A_setup()

    def _B_setup():
        B, S, D = 1, 2048, 1024
        ks = 4
        return {
            "q": _w((lambda *s: _rng.normal(s) * 0.05)(B, S, D)),
            "k": _w((lambda *s: _rng.normal(s) * 0.8)(B, S, D)),
            "v": _w((lambda *s: _rng.normal(s) * 0.8)(B, S, D)),
            "shift_k": _w((lambda *s: _rng.normal(s) * 0.8)(D, ks) * 0.5),
            "ssm_k": _w((lambda *s: _rng.normal(s) * 0.8)(D, S) * (1.0 / S ** 0.5)),
            "ssm_D": _w((lambda *s: _rng.normal(s) * 0.8)(D)),
        }
    _B_in = _B_setup()

    return {
        "A_x": _A_in["x"],
        "A_c_kv": _A_in["c_kv"],
        "A_w_q": _A_in["w_q"],
        "A_w_uk": _A_in["w_uk"],
        "A_w_uv": _A_in["w_uv"],
        "A_w_o": _A_in["w_o"],
        "B_q": _B_in["q"],
        "B_k": _B_in["k"],
        "B_v": _B_in["v"],
        "B_shift_k": _B_in["shift_k"],
        "B_ssm_k": _B_in["ssm_k"],
        "B_ssm_D": _B_in["ssm_D"],
        "gate_w": _w((lambda *s: _rng.normal(s) * 0.05)(1024) * 16.0),
    }

def reference(A_x, A_c_kv, A_w_q, A_w_uk, A_w_uv, A_w_o, B_q, B_k, B_v, B_shift_k, B_ssm_k, B_ssm_D, gate_w):
    def _A_ref(x, c_kv, w_q, w_uk, w_uv, w_o):
        B, Sq, M = x.shape[0], x.shape[1], x.shape[2]
        Sk = c_kv.shape[1]
        H, D = w_q.shape[1], w_q.shape[2]
        q = jnp.einsum("bqm,mhd->bhqd", x, w_q)
        k = jnp.einsum("bkc,chd->bhkd", c_kv, w_uk)
        v = jnp.einsum("bkc,chd->bhkd", c_kv, w_uv)
        scores = jnp.einsum("bhqd,bhkd->bhqk", q, k) * (D ** -0.5)
        off = Sk - Sq
        qi = jnp.arange(Sq)[:, None]
        kj = jnp.arange(Sk)[None, :]
        cmask = kj <= (qi + off)
        scores = jnp.where(cmask[None, None], scores, -1e9)
        p = _softmax(scores, axis=-1)
        ctx = jnp.einsum("bhqk,bhkd->bhqd", p, v)
        return jnp.einsum("bhqd,hdm->bqm", ctx, w_o)

    def _B_ref(q, k, v, shift_k, ssm_k, ssm_D):
        B, S, D = q.shape
        ks = shift_k.shape[-1]
        k_pad = jnp.pad(k, ((0, 0), (ks - 1, 0), (0, 0)))
        k_shift = jnp.zeros_like(k)
        for t in range(ks):
            k_shift = k_shift + k_pad[:, t:t + S, :] * shift_k[:, ks - 1 - t][None, None, :]
        kv = k_shift * v
        L = 2 * S
        kv_pad = jnp.pad(kv, ((0, 0), (0, S), (0, 0)))
        kf_pad = jnp.pad(ssm_k, ((0, 0), (0, S)))
        kv_f = (lambda x, axes=(-2,-1): jnp.fft.rfft2(x.astype(jnp.float32), axes=axes))(kv_pad[:, None, :, :], axes=(1, 2))
        kf_f = (lambda x, axes=(-2,-1): jnp.fft.rfft2(x.astype(jnp.float32), axes=axes))(kf_pad[:, None, :], axes=(1, 2))
        kf_f = (lambda x, *d: x.transpose(*d))(kf_f, 1, 2, 0)
        y_f = kv_f * kf_f[None, :, :, :]
        y = (lambda x, s, axes=(-2,-1): jnp.fft.irfft2(x, s=s, axes=axes).astype(jnp.bfloat16))(y_f, (1, L), axes=(1, 2))[:, 0, :S, :]
        y = y + kv * ssm_D[None, None, :]
        return q * y

    x = A_x
    g = _sigmoid((x * gate_w).sum(-1, keepdims=True))
    a = _A_ref(x, A_c_kv, A_w_q, A_w_uk, A_w_uv, A_w_o)
    b = _B_ref(x, B_k, B_v, B_shift_k, B_ssm_k, B_ssm_D)
    return g * a + (1 - g) * b
```

```python
import jax
import jax.numpy as jnp
import numpy as np
from jax import lax
from jax.experimental import pallas as pl
from jax.experimental.pallas import tpu as pltpu


S, M, DC, H, D = 2048, 1024, 512, 32, 128
C = 128
NC = S // C
BQ = 256
NB = S // BQ
NBUF = 3
f32, bf16, i32, u32 = jnp.float32, jnp.bfloat16, jnp.int32, jnp.uint32
NT = (((1,), (1,)), ((), ()))
QSCALE = float(D ** -0.5 * np.log2(np.e))
PACE = 4.0
LEAD = 300
MACANCH = "none"
PH = "123"
QR = 128
LAG = 2


def _dft_matrices():
    k = np.arange(C)[:, None]
    t = np.arange(C)[None, :]
    ang = 2 * np.pi * (k + 0.25) * t / C
    fwd = np.stack([np.cos(ang).reshape(16, 8, C), np.sin(ang).reshape(16, 8, C)], axis=1).reshape(2 * C, C)
    inv = fwd.T / C
    return fwd.astype(bf16), np.ascontiguousarray(inv).astype(bf16)


_FWD, _INV = _dft_matrices()


class _Clock:
    def __init__(self, zero):
        self.t = 0.0
        self.marks = []
        self.zv = jnp.full((8, 128), zero, i32)

    def note(self, val, cycles):
        n = val.shape[0] // 8
        for a in range(n):
            self.marks.append((self.t + cycles * (a + 1) / n, val, a * 8))
        self.t += cycles

    def token(self, when):
        _, val, a = [m for m in self.marks if m[0] <= when][-1]
        return pltpu.bitcast(val[a:a + 8, :128], i32) & self.zv

    def after(self, x, when):
        return pltpu.bitcast(pltpu.bitcast(x, i32) | self.token(when), f32)

    def dot(self, a, b):
        out = jnp.dot(a, b, preferred_element_type=f32)
        self.note(out, a.shape[0] * a.shape[1] * b.shape[1] / (512 * 128))
        return out

    def kdot(self, lhs, rhs, K):
        acc = None
        for c in range(0, K, 512):
            c1 = min(c + 512, K)
            part = self.dot(lhs(c, c1), rhs(c, c1))
            acc = part if acc is None else acc + part
        return acc


def _split_heads(u):
    return pltpu.bitcast(u << 16, f32), pltpu.bitcast(u & np.uint32(0xFFFF0000), f32)


def _lhs_terms(a11, a12, a21, a22):
    return (a11 + a22, a21 + a22, a11, a22, a11 + a12, a21 - a11, a12 - a22)


def _rhs_terms(b11, b12, b21, b22):
    return (b11 + b22, b11, b12 - b22, b21 - b11, b22, b11 + b12, b21 + b22)


def _strassen(prod, order=(5, 6, 0, 1, 2, 3, 4)):
    m = {}
    for t in order:
        m[t] = prod(t)
    return (m[0] + m[6] + m[3] - m[4], m[2] + m[4], m[1] + m[3], m[0] + m[5] - m[1] + m[2])


def _kernel(x_hbm, c_hbm, wq_hbm, wk_hbm, wv_hbm, wo_hbm, bk_hbm, bv_hbm, hk_hbm,
            shift_hbm, dd_hbm, gw_hbm, fwd_hbm, inv_hbm, o_hbm,
            x_s, xt, c_s, ct, wo_s, wot, ctx, yb, o_s,
            bk_s, bv_s, hk_s, wqraw, wqt, xsp, hsp, qsp,
            wkraw, wvraw, wkvt, q_s, k_s, v_s, at, cap, small, fwd_s, inv_s, kpad, *rest):
    sb, pb, lb = rest[:NBUF], rest[NBUF:2 * NBUF], rest[2 * NBUF:3 * NBUF]
    shift_s, dd_s, gw_s, sem, osem = rest[3 * NBUF:]
    copy = pltpu.make_async_copy

    def x_copy(r):
        rows = pl.ds(r * (S // 4), S // 4)
        return copy(x_hbm.at[rows], x_s.at[rows], sem.at[r])

    c_copy = copy(c_hbm, c_s, sem.at[4])
    wo_copy = copy(wo_hbm, wo_s, sem.at[5])
    small_copies = [copy(a, b, sem.at[20 + n]) for n, (a, b) in enumerate(
        ((shift_hbm, shift_s), (dd_hbm, dd_s), (gw_hbm, gw_s), (fwd_hbm, fwd_s), (inv_hbm, inv_s)))]

    def kv_copies(j):
        return (copy(wk_hbm.bitcast(u32).at[:, j, :], wkraw.at[j % 2], sem.at[6 + j % 2]),
                copy(wv_hbm.bitcast(u32).at[:, j, :], wvraw.at[j % 2], sem.at[8 + j % 2]))

    def p1_copies(cb):
        cols = pl.ds(pl.multiple_of(cb * 128, 128), 128)
        s = cb % 2
        return (copy(hk_hbm.at[cols, :], hk_s.at[s], sem.at[10 + s]),
                copy(bk_hbm.at[:, cols], bk_s.at[s], sem.at[12 + s]),
                copy(bv_hbm.at[:, cols], bv_s.at[s], sem.at[14 + s]),
                copy(wq_hbm.bitcast(u32).at[:, 2 * cb, :], wqraw.at[s, 0], sem.at[16 + s]),
                copy(wq_hbm.bitcast(u32).at[:, 2 * cb + 1, :], wqraw.at[s, 1], sem.at[18 + s]))

    def lhs_prep(src, dst, blk, kh):
        top, bot = slice(blk * 256, blk * 256 + 128), slice(blk * 256 + 128, blk * 256 + 256)
        terms = _lhs_terms(src[top, :kh].astype(f32), src[top, kh:].astype(f32),
                           src[bot, :kh].astype(f32), src[bot, kh:].astype(f32))
        for n, t in enumerate((0, 1, 4, 5, 6)):
            dst[n, blk * 128:(blk + 1) * 128, :] = terms[t].astype(bf16)

    def lhs_term(src, dst, t, r0, rows, kh):
        top = (r0 // 128) * 256 + r0 % 128
        if t == 2:
            return src[top:top + rows, :kh]
        if t == 3:
            return src[top + 128:top + 128 + rows, kh:]
        return dst[(0, 1, 4, 5, 6).index(t), r0:r0 + rows, :]

    def phase1(it, _):
        @pl.when(it < 7)
        def _():
            for cp in p1_copies(it + 1):
                cp.start()

        @pl.when(it == 2)
        def _():
            wo_copy.start()

        @pl.when(it == 4)
        def _():
            c_copy.start()
            for cp in kv_copies(0):
                cp.start()

        with jax.named_scope('w1'):
            for cp in p1_copies(it):
                cp.wait()

        zero = it // 64
        clk = _Clock(zero)
        s = it % 2
        fwd = fwd_s[...]
        for m in range(NC):
            hsp[m] = lax.dot_general(fwd, hk_s[s, :, m * C:(m + 1) * C], NT, preferred_element_type=f32)
        kpad[8:8 + S, :] = bk_s[s].astype(f32)
        taps = [small[it, j:j + 1, :] for j in range(4)]
        for j in range(NC):
            ks = sum(kpad[8 - t + j * C:8 - t + (j + 1) * C, :] * taps[t] for t in range(4))
            kv = (ks * bv_s[s, j * C:(j + 1) * C, :].astype(f32)).astype(bf16)
            xsp[j] = jnp.dot(fwd, kv, preferred_element_type=f32)
        for p in range(2):
            b11, b12 = _split_heads(wqraw[s, p, :M // 2, :])
            b21, b22 = _split_heads(wqraw[s, p, M // 2:, :])
            for t, term in enumerate(_rhs_terms(b11, b12, b21, b22)):
                wqt[p, t] = term.astype(bf16)
            for r0 in range(0, S // 2, QR):
                cs = _strassen(lambda t: clk.dot(lhs_term(x_s, xt, t, r0, QR, M // 2), wqt[p, t]))
                top = (r0 // 128) * 256 + r0 % 128
                for n, cc in enumerate(cs):
                    row = top + 128 * (n // 2)
                    ctx[4 * it + 2 * p + n % 2, row:row + QR, :] = (cc * QSCALE).astype(bf16)
        dvec = small[it, 4:5, :]
        for f in range(16):
            re, im = slice(16 * f, 16 * f + 8), slice(16 * f + 8, 16 * f + 16)
            zz = zero
            if MACANCH == "scalar":
                zz = clk.token(16 + (clk.t - 1000) * f / 16)[0, 0]
            hv, xv = hsp.at[pl.ds(zz, NC)], xsp.at[pl.ds(zz, NC)]
            hr = [hv[m, re, :] for m in range(NC)]
            hi = [hv[m, im, :] for m in range(NC)]
            hr[0] = hr[0] + dvec
            xr = [xv[j, re, :] for j in range(NC)]
            xi = [xv[j, im, :] for j in range(NC)]
            pr = pi = None
            for i in range(NC):
                ar = ai = None
                for j in range(i + 1):
                    tr = hr[i - j] * xr[j] - hi[i - j] * xi[j]
                    ti = hr[i - j] * xi[j] + hi[i - j] * xr[j]
                    ar = tr if ar is None else ar + tr
                    ai = ti if ai is None else ai + ti
                qr, qi = (ar, ai) if pr is None else (ar + pi, ai - pr)
                pr, pi = ar, ai
                qsp[i, 16 * f:16 * f + 16, :] = jnp.concatenate([qr, qi], axis=0).astype(bf16)
        inv = inv_s[...]
        for i in range(NC):
            yb[it, i * C:(i + 1) * C, :] = jnp.dot(inv, qsp[i], preferred_element_type=f32)

    def phase2(g, _):
        @pl.when(g < H // 2 - 1)
        def _():
            for cp in kv_copies(g + 1):
                cp.start()

        for cp in kv_copies(g):
            cp.wait()

        z = g // 64
        z8 = pl.multiple_of(z * 8, 8)
        clk = _Clock(z)
        done = {}
        for n, raw in enumerate((wkraw, wvraw)):
            b11, b12 = _split_heads(raw[g % 2, :DC // 2, :])
            b21, b22 = _split_heads(raw[g % 2, DC // 2:, :])
            for t, term in enumerate(_rhs_terms(b11, b12, b21, b22)):
                wkvt[t, n] = term.astype(bf16)
        for e in range(2):
            q_s[e] = ctx[2 * g + e]

        def proj(i):
            cs = _strassen(lambda t: clk.dot(lhs_term(c_s, ct, t, i * 128, 128, DC // 2),
                                             jnp.concatenate([wkvt[t, 0], wkvt[t, 1]], axis=1)))
            for n, cc in enumerate(cs):
                r = slice(i * BQ + 128 * (n // 2), i * BQ + 128 * (n // 2) + 128)
                k_s[n % 2, r, :] = cc[:, :D].astype(bf16)
                v_s[n % 2, r, :] = cc[:, D:].astype(bf16)

        def chunks(i):
            nfull = i * BQ + 128
            out = [(0, c, min(c + 512, nfull)) for c in range(0, nfull, 512)]
            out += [(t * 128, i * BQ + t * 128, i * BQ + (t + 1) * 128) for t in range(1, BQ // 128)]
            return out

        def qk(u):
            i, e = divmod(u, 2)
            sbuf = sb[u % NBUF]
            for n, (r0, c0, c1) in enumerate(chunks(i)):
                s = lax.dot_general(q_s[e, i * BQ + r0:(i + 1) * BQ, :], k_s[e, c0:c1, :], NT,
                                    preferred_element_type=f32)
                ts = [s[:, c:c + 128] for c in range(0, c1 - c0, 128)]
                if c1 == i * BQ + r0 + 128:
                    d = jnp.minimum(ts[-1][:128], cap[...])
                    ts[-1] = d if ts[-1].shape[0] == 128 else jnp.concatenate([d, ts[-1][128:]], axis=0)
                mx = ts[0]
                for tt in ts[1:]:
                    mx = jnp.maximum(mx, tt)
                clk.note(ts[-1], (BQ - r0) * (c1 - c0) / 512)
                for j, tt in enumerate(ts):
                    sbuf[r0:BQ, c0 + j * 128:c0 + (j + 1) * 128] = tt
                if len(ts) > 1:
                    sbuf[r0:BQ, S + n * 128:S + (n + 1) * 128] = mx
            done[u] = clk.t

        def sm(u):
            i = u // 2
            sv = sb[u % NBUF].at[pl.ds(z8, BQ)]
            for r0 in range(0, BQ, 8):
                L = i * BQ + (r0 // 128 + 1) * 128
                r = slice(r0, r0 + 8)
                mx = None
                for n, (q0, c0, c1) in enumerate(chunks(i)):
                    if q0 <= r0:
                        a = S + n * 128 if c1 - c0 > 128 else c0
                        mx = sv[r, a:a + 128] if mx is None else jnp.maximum(mx, sv[r, a:a + 128])
                t0 = done[u]
                t1 = max(t0, min(clk.t - LEAD, t0 + PACE * (2 * i + 1.5) * BQ // 8))
                mx = clk.after(mx, t0 + (t1 - t0) * r0 / BQ)
                m = jnp.max(mx, axis=1, keepdims=True)
                ps = [jnp.exp2(sv[r, c:c + 128] - m) for c in range(0, L, 128)]
                ls = ps[0]
                for p in ps[1:]:
                    ls = ls + p
                l = jnp.sum(ls, axis=1, keepdims=True)
                linv = pltpu.reciprocal(l, approx=True)
                linv = linv * (2.0 - l * linv)
                lb[u % NBUF][r, :] = jnp.broadcast_to(linv, (8, 128))
                ps[0] = jnp.maximum(ps[0], -linv)
                for j in range(0, len(ps), 2):
                    pp = jnp.concatenate(ps[j:j + 2], axis=1)
                    pb[u % NBUF][r, j * 128:j * 128 + pp.shape[1]] = pp.astype(bf16)

        def pv(u):
            i, e = divmod(u, 2)
            lv = lb[u % NBUF].at[pl.ds(z8, BQ)]
            for r0 in range(0, BQ, 128):
                L = i * BQ + r0 + 128
                r = slice(r0, r0 + 128)
                o = clk.kdot(lambda a, b: pb[u % NBUF][r, a:b], lambda a, b: v_s[e, a:b, :], L)
                ctx[2 * g + e, i * BQ + r0:i * BQ + r0 + 128, :] = (o * lv[r, :]).astype(bf16)

        proj(0)
        for u in range(2 * NB + LAG):
            if u % 2 == 0 and u // 2 + 1 < NB:
                proj(u // 2 + 1)
            if u < 2 * NB:
                qk(u)
            if u >= LAG:
                sm(u - LAG)
                pv(u - LAG)

        top = pl.ds(pl.multiple_of(g * D, D), D)
        bot = pl.ds(pl.multiple_of(g * D + H * D // 2, D), D)
        terms = _rhs_terms(wo_s[top, :M // 2].astype(f32), wo_s[top, M // 2:].astype(f32),
                           wo_s[bot, :M // 2].astype(f32), wo_s[bot, M // 2:].astype(f32))
        for n, t in enumerate((0, 2, 3, 5, 6)):
            wot[n, top, :] = terms[t].astype(bf16)

    def o_copy(r):
        rows = pl.ds(pl.multiple_of(r * 256, 256), 256)
        return copy(o_s.at[rows], o_hbm.at[rows], osem.at[r])

    def phase3(r, _):
        halves = [pl.ds(pl.multiple_of(r * 256 + 128 * e, 128), 128) for e in range(2)]
        for hd in range(H // 2):
            terms = _lhs_terms(ctx[hd, halves[0], :].astype(f32), ctx[hd + H // 2, halves[0], :].astype(f32),
                               ctx[hd, halves[1], :].astype(f32), ctx[hd + H // 2, halves[1], :].astype(f32))
            for n, t in enumerate((0, 1, 4, 5, 6)):
                at[n, hd] = terms[t].astype(bf16)

        def lhs(t):
            if t == 2:
                parts = [ctx[hd, halves[0], :] for hd in range(H // 2)]
            elif t == 3:
                parts = [ctx[hd + H // 2, halves[1], :] for hd in range(H // 2)]
            else:
                parts = [at[(0, 1, 4, 5, 6).index(t), hd] for hd in range(H // 2)]
            return jnp.concatenate(parts, axis=1)

        def rhs(t, n0, n1):
            if t == 1:
                return wo_s[:H * D // 2, n0:n1]
            if t == 4:
                return wo_s[H * D // 2:, M // 2 + n0:M // 2 + n1]
            return wot[(0, 2, 3, 5, 6).index(t), :, n0:n1]

        gw = gw_s[...].astype(f32)
        gates = []
        for rows in halves:
            xf = x_s[rows, :].astype(f32)
            logit = sum(xf[:, n * 128:(n + 1) * 128] * gw[n:n + 1, :] for n in range(8))
            gates.append(jax.nn.sigmoid(jnp.sum(logit, axis=1, keepdims=True)))
        NW = 128
        for n0 in range(0, M // 2, NW):
            cs = _strassen(lambda t: jnp.dot(lhs(t), rhs(t, n0, n0 + NW), preferred_element_type=f32),
                           order=(2, 3, 1, 4, 0, 5, 6))
            for n, a in enumerate(cs):
                rows, gate, c0 = halves[n // 2], gates[n // 2], n0 + (n % 2) * (M // 2)
                y = jnp.concatenate([yb[c // 128, rows, :] for c in range(c0, c0 + NW, 128)], axis=1)
                b = x_s[rows, c0:c0 + NW].astype(f32) * y
                o_s[rows, c0:c0 + NW] = (gate * a + (1.0 - gate) * b).astype(bf16)
        o_copy(r).start()

    for cp in small_copies:
        cp.start()
    for r in range(4):
        x_copy(r).start()
    if "1" in PH:
        for cp in p1_copies(0):
            cp.start()
    else:
        wo_copy.start()
        c_copy.start()
        for cp in kv_copies(0):
            cp.start()
    row = lax.broadcasted_iota(i32, (128, 128), 0)
    col = lax.broadcasted_iota(i32, (128, 128), 1)
    cap[...] = jnp.where(col <= row, jnp.inf, -1e30)
    kpad[0:8, :] = jnp.zeros((8, 128), f32)
    for cp in small_copies:
        cp.wait()
    sh = shift_s[...].astype(f32)
    dd = dd_s[...].astype(f32)
    for cb in range(8):
        small[cb, 0:4, :] = sh[:, cb * 128:(cb + 1) * 128]
        small[cb, 4:5, :] = dd[cb:cb + 1, :]
    for r in range(4):
        x_copy(r).wait()
        lhs_prep(x_s, xt, 2 * r, M // 2)
        lhs_prep(x_s, xt, 2 * r + 1, M // 2)
    if "1" in PH:
        with jax.named_scope('ph1'):
            lax.fori_loop(0, 8, phase1, None)
    c_copy.wait()
    wo_copy.wait()
    for blk in range(NB):
        lhs_prep(c_s, ct, blk, DC // 2)
    if "2" in PH:
        with jax.named_scope('ph2'):
            lax.fori_loop(0, H // 2, phase2, None)
    else:
        for cp in kv_copies(0):
            cp.wait()
    if "3" in PH:
        with jax.named_scope('ph3'):
            lax.fori_loop(0, S // 256, phase3, None)
        for r in range(S // 256):
            o_copy(r).wait()
    else:
        zz = gw_s[...].astype(f32)[0, 0].astype(i32)
        o_s[0:128, 0:128] = (ctx[zz, 0:128, :].astype(f32) + yb[zz, 0:128, :] + wot[zz, 0:128, 0:128].astype(f32)).astype(bf16)
        o_copy(0).start()
        o_copy(0).wait()


@jax.jit
def pallas_gated_mix__compressed_kv_cla__ssm_conv_h3__prompt_kernel(
        A_x, A_c_kv, A_w_q, A_w_uk, A_w_uv, A_w_o, B_q, B_k, B_v, B_shift_k, B_ssm_k, B_ssm_D, gate_w):
    del B_q
    hbm = pl.BlockSpec(memory_space=pl.ANY)
    vm = pltpu.VMEM
    out = pl.pallas_call(
        _kernel,
        in_specs=[hbm] * 14,
        out_specs=hbm,
        out_shape=jax.ShapeDtypeStruct((S, M), bf16),
        scratch_shapes=[
            vm((S, M), bf16), vm((5, S // 2, M // 2), bf16),
            vm((S, DC), bf16), vm((5, S // 2, DC // 2), bf16),
            vm((H * D, M), bf16), vm((5, H * D // 2, M // 2), bf16),
            vm((H, S, D), bf16), vm((8, S, 128), f32), vm((S, M), bf16),
            vm((2, S, 128), bf16), vm((2, S, 128), bf16), vm((2, 128, S), bf16),
            vm((2, 2, M, D), u32), vm((2, 7, M // 2, D), bf16),
            vm((NC + 1, 2 * C, 128), f32), vm((NC + 1, 2 * C, 128), f32), vm((NC, 2 * C, 128), bf16),
            vm((2, DC, D), u32), vm((2, DC, D), u32), vm((7, 2, DC // 2, D), bf16),
            vm((2, S, D), bf16), vm((2, S, D), bf16), vm((2, S, D), bf16),
            vm((5, H // 2, 128, D), bf16),
            vm((128, 128), f32), vm((8, 32, 128), f32),
            vm((2 * C, C), bf16), vm((C, 2 * C), bf16), vm((S + 32, 128), f32),
            *([vm((BQ + 8, S + 512), f32)] * NBUF + [vm((BQ, S), bf16)] * NBUF + [vm((BQ + 32, 128), f32)] * NBUF),
            vm((4, M), bf16), vm((8, 128), bf16), vm((8, 128), bf16),
            pltpu.SemaphoreType.DMA((25,)), pltpu.SemaphoreType.DMA((8,)),
        ],
        compiler_params=pltpu.CompilerParams(vmem_limit_bytes=118 * 2**20),
    )(A_x.reshape(S, M), A_c_kv.reshape(S, DC), A_w_q, A_w_uk, A_w_uv, A_w_o.reshape(H * D, M),
      B_k.reshape(S, M), B_v.reshape(S, M), B_ssm_k,
      B_shift_k.T, B_ssm_D.reshape(8, 128), gate_w.reshape(8, 128), _FWD, _INV)
    return out.reshape(1, S, M)
```

```python
import jax
import jax.numpy as jnp
import numpy as np
from jax import lax
from jax.experimental import pallas as pl
from jax.experimental.pallas import tpu as pltpu

S, M, DC, H, D = 2048, 1024, 512, 32, 128
C = 128
NC = S // C
BQ = 256
NB = S // BQ
NG = H // 2
NBUF = 3
f32, bf16, i32, u32 = jnp.float32, jnp.bfloat16, jnp.int32, jnp.uint32
NN = (((1,), (0,)), ((), ()))
NT = (((1,), (1,)), ((), ()))
QSCALE = float(D ** -0.5 * np.log2(np.e))


def _dft_matrices():
    k = np.arange(C)[:, None]
    t = np.arange(C)[None, :]
    ang = 2 * np.pi * (k + 0.25) * t / C
    fwd = np.stack([np.cos(ang).reshape(16, 8, C), np.sin(ang).reshape(16, 8, C)], axis=1).reshape(2 * C, C)
    inv = np.concatenate([fwd.T[:, :C], fwd.T[:, C:]], axis=0) / C
    return fwd.astype(bf16), inv.astype(bf16)


_FWD, _INV = _dft_matrices()

_LHS = (((0, 1), (3, 1)), ((2, 1), (3, 1)), ((0, 1),), ((3, 1),),
        ((0, 1), (1, 1)), ((2, 1), (0, -1)), ((1, 1), (3, -1)))
_RHS = (((0, 1), (3, 1)), ((0, 1),), ((1, 1), (3, -1)), ((2, 1), (0, -1)),
        ((3, 1),), ((0, 1), (1, 1)), ((2, 1), (3, 1)))
_OUT = (((0, 1), (6, 1), (3, 1), (4, -1)), ((2, 1), (4, 1)), ((1, 1), (3, 1)),
        ((0, 1), (5, 1), (1, -1), (2, 1)))
_ORDER = (1, 4, 2, 5, 0, 3, 6)


def _signed_sum(terms, get):
    acc = get(terms[0][0])
    for idx, sign in terms[1:]:
        acc = acc + get(idx) if sign > 0 else acc - get(idx)
    return acc


def _output(n, get, order):
    terms = sorted(_OUT[n], key=lambda term: order.index(term[0]))
    if terms[0][1] < 0:
        terms[:2] = terms[1], terms[0]
    return _signed_sum(terms, get)


def _operands(table, quads):
    return [_signed_sum(terms, lambda n: quads[n]) for terms in table]


def _operands2(table, outer, block):
    return _operands(table, [
        _signed_sum(table[outer], lambda n: block(2 * (n // 2) + i, 2 * (n % 2) + j))
        for i in range(2) for j in range(2)])


def _finished(order):
    last = [max(order.index(t) for t, _ in terms) for terms in _OUT]
    return [[n for n in range(4) if last[n] == pos] for pos in range(7)]


def _strassen(prod, order):
    m = {t: prod(t) for t in order}
    return [_output(n, lambda t: m[t], order) for n in range(4)]


def _strassen2(prod, emit, order, quadrant_done=lambda n: None):
    m = {}
    for o, done in zip(order, _finished(order)):
        m[o] = _strassen(lambda t: prod(o, t), order)
        for q in done:
            for n in sum(_finished(order), []):
                emit(2 * (q // 2) + n // 2, 2 * (q % 2) + n % 2, _output(q, lambda t: m[t][n], order))
            quadrant_done(q)


class _Clock:
    def __init__(self, zero=None):
        self.busy = [0, 0, 0, 0]
        self.marks = []
        self.jobs = []
        if zero is not None:
            self.zero = jnp.full((8, 128), zero, i32)

    @property
    def t(self):
        return min(self.busy)

    def advance(self, rows, tiles):
        for _ in range(tiles):
            u = self.busy.index(min(self.busy))
            begin = self.busy[u]
            self.busy[u] += rows
        return begin

    def run_due(self, when):
        ready = [j for j in self.jobs if j[0] < when]
        self.jobs = [j for j in self.jobs if j[0] >= when]
        out = [(t, job()) for t, job in ready]
        return [o for o in out if o[1] is not None]

    def dot(self, a, b, dims=NN):
        rows, first = a.shape[0], self.t
        ready = self.run_due(first + rows)
        if ready:
            words = pltpu.bitcast(a[:, :128], i32)
            parts = [words[r:r + 8] for r in range(0, rows // 2, 8)]
            for t, val in ready:
                n = int(max(t - first, 0)) // 16
                parts[n] = parts[n] | (pltpu.bitcast(val, i32) & self.zero)
            head = pltpu.bitcast(jnp.concatenate(parts, axis=0), bf16)
            a = head if a.shape[1] == 128 else jnp.concatenate([head, a[:, 128:]], axis=1)
        out = lax.dot_general(a, b, dims, preferred_element_type=f32)
        begin = self.advance(rows, a.shape[1] // 128)
        self.marks += [(begin + r + 8, out, r) for r in range(0, rows, 8)]
        return out

    def after(self, when):
        _, val, r = max((m for m in self.marks if m[0] <= max(when, 8)), key=lambda m: m[0])
        nothing = pltpu.bitcast(val[r:r + 8, :], i32) & self.zero

        def hold(x):
            words = pltpu.bitcast(x, i32)
            return pltpu.bitcast(words | jnp.concatenate([nothing] * (words.shape[0] // 8), axis=0), x.dtype)
        return hold


PACE, MINPACE, WINDOW = 5.45, 3.9, 780


def _attention_plan():
    steps = [("k", 0), ("k", 1)]
    for u in range(2 * NB + NBUF - 1):
        if u < 2 * NB:
            steps.append(("qk", u))
        if u % 2 == 0 and 1 < u // 2 + 1 < NB:
            steps.append(("k", u // 2 + 1))
        if u % 2 == 1 and u < 2 * NB:
            steps.append(("v", u // 2))
        if u >= NBUF - 1:
            steps.append(("pv", u - NBUF + 1))
    clk, scored, needed = _Clock(), {}, {}
    for kind, u in steps:
        if kind == "qk":
            clk.advance(BQ, u // 2 * 2 + 1)
            clk.advance(128, 1)
            scored[u] = max(clk.busy)
        elif kind == "pv":
            for half in range(2):
                needed[u, half] = clk.t
                clk.advance(128, u // 2 * 2 + 1 + half)
        else:
            clk.advance(128, 14)
    groups = [(u, r) for u in range(2 * NB) for r in range(0, BQ, 8)]
    work = [u // 2 * 2 + 1 + r // 128 for u, r in groups]
    times, t = [], 0
    for (u, r), w in zip(groups, work):
        t = max(t, scored[u])
        times.append(t)
        t += PACE * w
    t = clk.t
    for n in reversed(range(len(groups))):
        u, r = groups[n]
        t = times[n] = min(times[n], needed[u, r // 128] - WINDOW, t - MINPACE * work[n])
    return steps, dict(zip(groups, times))


def _as_bf16(words):
    return pltpu.bitcast(words, bf16)


def _head(words, e):
    return pltpu.bitcast(words & np.uint32(0xFFFF0000) if e else words << 16, f32)


def _kernel(x_hbm, c_hbm, wq_hbm, wk_hbm, wv_hbm, wo_hbm, bk_hbm, bv_hbm, hk_hbm,
            shift_hbm, dd_hbm, gw_hbm, fwd_hbm, inv_hbm, o_hbm,
            x_s, xt, c_s, ct, wo_s, wot, ctx, yb, o_s, gate_s,
            bk_s, bv_s, hk_s, wq_s, xsp, hsp, qsp, kpad,
            wk_s, wv_s, wkt, wvt, q_s, k_s, v_s, cap, coef, fwd_s, inv_s,
            wqt, sb, pb, lb, at, shift_s, dd_s, gw_s, sem, osem):
    copy = pltpu.make_async_copy

    def start(copies):
        for cp in copies:
            cp.start()

    def wait(copies):
        for cp in copies:
            cp.wait()

    def x_copy(r):
        rows = pl.ds(pl.multiple_of(r * 512, 512), 512)
        return [copy(x_hbm.at[rows], x_s.at[rows], sem.at[r])]

    c_copy = [copy(c_hbm, c_s, sem.at[4])]
    small_copies = [copy(a, b, sem.at[5 + n]) for n, (a, b) in enumerate(
        ((shift_hbm, shift_s), (dd_hbm, dd_s), (gw_hbm, gw_s), (fwd_hbm, fwd_s), (inv_hbm, inv_s)))]

    def phase1_copies(n):
        cols = pl.ds(pl.multiple_of(n * 128, 128), 128)
        s = n & 1
        return [copy(hk_hbm.at[cols, :], hk_s.at[s], sem.at[10 + s]),
                copy(bk_hbm.at[:, cols], bk_s.at[s], sem.at[12 + s]),
                copy(bv_hbm.at[:, cols], bv_s.at[s], sem.at[14 + s]),
                copy(wq_hbm.bitcast(u32).at[:, 2 * n, :], wq_s.at[s, 0], sem.at[16 + s]),
                copy(wq_hbm.bitcast(u32).at[:, 2 * n + 1, :], wq_s.at[s, 1], sem.at[18 + s])]

    def kv_copies(g):
        return [copy(wk_hbm.bitcast(u32).at[:, g, :], wk_s.at[g & 1], sem.at[20 + (g & 1)]),
                copy(wv_hbm.bitcast(u32).at[:, g, :], wv_s.at[g & 1], sem.at[22 + (g & 1)])]

    def wo_copy(g):
        src = wo_hbm.at[pl.ds((g >> 1) * 4, 4), pl.ds(pl.multiple_of((g & 1) * 64, 64), 64), :]
        return [copy(src, wo_s.at[g & 1], sem.at[24 + (g & 1)])]

    def q_copy(g):
        return [copy(ctx.at[pl.ds(2 * g, 2)], q_s.at[g & 1], sem.at[26 + (g & 1)])]

    def o_copy(r, half):
        rows, cols = pl.ds(pl.multiple_of(r * 512, 512), 512), pl.ds(half * 512, 512)
        return [copy(o_s.at[rows, cols], o_hbm.at[rows, cols], osem.at[2 * r + half])]

    def lhs_operand(ref, t, blk):
        words = ref.bitcast(u32)
        return _as_bf16(jnp.concatenate([words[t, c, blk * 64:(blk + 1) * 64, :] for c in range(2)], axis=1))

    def kv_weight_prep(raw, dst, hold_at=lambda frac: (lambda x: x)):
        for r in range(0, DC // 2, 16):
            hold = hold_at(r / (DC // 2))
            words = [hold(raw[a:a + 16, :]) for a in (r, DC // 2 + r)]
            for t, term in enumerate(_operands(_RHS, [_head(w, e) for w in words for e in range(2)])):
                dst[t, r:r + 16, :] = term.astype(bf16)


    def phase1(it, _):
        @pl.when(it > 0)
        def _():
            wait(phase1_copies(it))

        zero = it >> 6
        clk = _Clock(zero)
        s = it & 1
        fwd = _as_bf16(fwd_s.bitcast(u32)[...])
        kpad[8:8 + S, :] = bk_s[s].astype(f32)
        taps = [coef[it, j:j + 1, :] for j in range(4)]
        for m in range(NC + 2):
            if m < NC:
                hsp[m] = clk.dot(fwd, hk_s[s, :, m * C:(m + 1) * C], NT)
            j = m - 2
            if j >= 0:
                ks = sum(kpad[8 - t + j * C:8 - t + (j + 1) * C, :] * taps[t] for t in range(4))
                kv = (ks * bv_s[s, j * C:(j + 1) * C, :].astype(f32)).astype(bf16)
                xsp[j] = clk.dot(fwd, kv)

        prepared = []

        def q_prod(blk, o, t):
            if o not in prepared:
                prepared.append(o)
                for r in range(0, M // 4, 16):
                    hold = clk.after(clk.t - 260 - 450 * (1 - r / (M // 4)))
                    terms = _operands2(_RHS, o, lambda k, hd: _head(
                        hold(wq_s[s, hd // 2, k * (M // 4) + r:k * (M // 4) + r + 16, :]), hd % 2))
                    for n, term in enumerate(terms):
                        wqt[o][n, r:r + 16, :] = term.astype(bf16)
            return clk.dot(lhs_operand(xt, 7 * o + t, blk), _as_bf16(wqt[o].bitcast(u32).at[pl.ds(zero, 7)][t]))

        for blk in range(S // 512):
            def q_emit(i, hd, val):
                ctx[4 * it + hd, blk * 512 + i * 128:blk * 512 + (i + 1) * 128, :] = val.astype(bf16)
            _strassen2(lambda o, t: q_prod(blk, o, t), q_emit, _ORDER)

        hsp[NC, :8, :] = clk.after(4400)(cap[:8, :])
        skip = coef[it, 4:5, :]
        hv, xv = hsp.at[pl.ds(zero, NC)], xsp.at[pl.ds(zero, NC)]
        for f in range(16):
            re, im = slice(16 * f, 16 * f + 8), slice(16 * f + 8, 16 * f + 16)
            hr = [hv[m, re, :] for m in range(NC)]
            hi = [hv[m, im, :] for m in range(NC)]
            hr[0] = hr[0] + skip
            xr = [xv[j, re, :] for j in range(NC)]
            xi = [xv[j, im, :] for j in range(NC)]
            pr = pi = None
            for i in range(NC):
                ar = ai = None
                for j in range(i + 1):
                    tr = hr[i - j] * xr[j] - hi[i - j] * xi[j]
                    ti = hr[i - j] * xi[j] + hi[i - j] * xr[j]
                    ar = tr if ar is None else ar + tr
                    ai = ti if ai is None else ai + ti
                qr, qi = (ar, ai) if pr is None else (ar + pi, ai - pr)
                pr, pi = ar, ai
                qsp[i, 16 * f:16 * f + 16, :] = jnp.concatenate([qr, qi], axis=0).astype(bf16)
        iw = inv_s.bitcast(u32)
        inv = _as_bf16(jnp.concatenate([iw[:C // 2, :], iw[C // 2:, :]], axis=1))
        qv = qsp.bitcast(u32).at[pl.ds(zero, NC)]
        for i in range(NC):
            yb[it, i * C:(i + 1) * C, :] = jnp.dot(inv, _as_bf16(qv[i]), preferred_element_type=f32)

        @pl.when(it < 6)
        def _():
            start(phase1_copies(it + 2))

        @pl.when(it == 6)
        def _():
            start(c_copy + wo_copy(0) + wo_copy(1) + kv_copies(0) + kv_copies(1))

    def phase2(g, _):
        @pl.when(g < NG - 1)
        def _():
            wait(kv_copies(g + 1))

        wait(wo_copy(g) + q_copy(g))
        zero = g >> 6
        first, second = (pl.ds(pl.multiple_of((g >> n) * 32, 32), BQ) for n in (7, 6))
        clk = _Clock(zero)
        qw = q_s.bitcast(u32).at[g & 1]
        steps, begin = _attention_plan()

        def up_project(i, wt, dst):
            out = _strassen(lambda t: clk.dot(lhs_operand(ct, t, i), _as_bf16(wt.bitcast(u32)[t])), _ORDER)
            for n, val in enumerate(out):
                r = i * BQ + 128 * (n // 2)
                dst[n % 2, r:r + 128, :] = val.astype(bf16)

        def scores(u):
            i, e = divmod(u, 2)
            for j in range(2 * i + 2):
                r0 = 128 if j == 2 * i + 1 else 0
                s = clk.dot(_as_bf16(qw[e, (i * BQ + r0) // 2:(i + 1) * BQ // 2, :]),
                            k_s[e, j * 128:(j + 1) * 128, :], NT)
                if j == 2 * i:
                    s = jnp.concatenate([jnp.minimum(s[:128], cap[...]), s[128:]], axis=0)
                if j == 2 * i + 1:
                    s = jnp.minimum(s, cap[...])
                sb[u % NBUF][r0:BQ, j * 128:(j + 1) * 128] = s
            for r0 in range(0, BQ, 8):
                clk.jobs.append((begin[u, r0] + WINDOW, lambda r0=r0: softmax(u, r0)))

        def softmax(u, r0):
            i = u // 2
            r = slice(r0, r0 + 8)
            cols = [slice(j * 128, (j + 1) * 128) for j in range(2 * i + 1 + r0 // 128)]
            s1, s2 = sb[u % NBUF].at[first], sb[u % NBUF].at[second]
            top = clk.after(begin[u, r0])(s1[r, cols[0]])
            for c in cols[1:]:
                top = jnp.maximum(top, s1[r, c])
            top = jnp.max(top, axis=1, keepdims=True)
            ps = [jnp.exp2(s2[r, c] - top) for c in cols]
            total = ps[0]
            for p in ps[1:]:
                total = total + p
            norm = pltpu.reciprocal(jnp.sum(total, axis=1, keepdims=True), full_range=False)
            norm = jnp.broadcast_to(norm, (8, 128))
            lb[u % NBUF][r, :] = norm * gate_s[i * BQ + r0:i * BQ + r0 + 8, :]
            short = u < 8
            if short:
                ps[0] = jnp.maximum(ps[0], -norm)
            for j in range(0, len(ps), 2):
                pair = jnp.concatenate(ps[j:j + 2], axis=1)
                pb[u % NBUF][r, j * 128:j * 128 + pair.shape[1]] = pair.astype(bf16)
            return None if short else norm

        def context(u):
            i, e = divmod(u, 2)
            for r0 in range(0, BQ, 128):
                clk.run_due(clk.t + 1)
                acc = None
                for j in range(2 * i + 1 + r0 // 128):
                    part = clk.dot(pb[u % NBUF][r0:r0 + 128, j * 128:(j + 1) * 128], v_s[e, j * 128:(j + 1) * 128, :])
                    acc = part if acc is None else acc + part
                row = i * BQ + r0
                ctx[2 * g + e, row:row + 128, :] = (acc * lb[u % NBUF].at[second][r0:r0 + 128, :]).astype(bf16)
                stored = ctx.bitcast(u32)[2 * g + e + zero, row // 2:row // 2 + 8, :]
                clk.jobs.append((max(clk.busy) + 400, lambda stored=stored: stored))

        for kind, u in steps:
            if kind == "k":
                up_project(u, wkt, k_s)
                k_done = clk.t
            elif kind == "v":
                up_project(u, wvt, v_s)
            elif kind == "qk":
                scores(u)
            else:
                context(u)

        kv_weight_prep(wk_s.at[(g + 1) & 1], wkt, lambda frac: clk.after(k_done + frac * 2000))
        kv_weight_prep(wv_s.at[(g + 1) & 1], wvt, lambda frac: clk.after(clk.t - 900 + frac * 600))
        wsrc = wo_s.at[g & 1]
        for r in range(0, 64, 16):
            out = pl.ds(pl.multiple_of(g * 64 + r, 16), 16)
            for c in range(2):
                for o in range(7):
                    hold = clk.after(((r // 8 + c) * 7 + o) * 24)
                    terms = _operands2(_RHS, o, lambda k, n: hold(
                        wsrc[k, r:r + 16, n * 256 + c * 128:n * 256 + (c + 1) * 128]).astype(f32))
                    for t, term in enumerate(terms):
                        wot[7 * o + t, c, out, :] = term.astype(bf16)

        @pl.when(g < NG - 3)
        def _():
            start(kv_copies(g + 3))

        @pl.when(g < NG - 2)
        def _():
            start(wo_copy(g + 2) + q_copy(g + 2))

    def phase3(r, _):
        zero = r >> 6
        clk = _Clock(zero)
        cv = ctx.bitcast(u32).at[:, pl.ds(pl.multiple_of(r * 256, 256), 256)]
        ww = wot.bitcast(u32)
        rows = pl.ds(pl.multiple_of(r * 512, 512), 512)
        yv, xv, gv, ov = yb.at[:, rows], x_s.at[rows], gate_s.at[rows], o_s.at[rows]
        plain = ((2, 2), (2, 3))
        prepared = []

        def prod(o, t):
            if (o, t) not in plain and o not in prepared:
                prepared.append(o)
                end = clk.t - 260
                for j in range(8):
                    for q in range(8):
                        hold = clk.after(end - min(end, 3000) * (1 - (j * 8 + q) / 64))
                        terms = _operands2(_LHS, o, lambda i, k: _as_bf16(
                            hold(cv[4 * j + k, 32 * q + 8 * i:32 * q + 8 * i + 8])).astype(f32))
                        for n, term in enumerate(terms):
                            if (o, n) not in plain:
                                at[len(prepared) & 1][n, j, 16 * q:16 * q + 16] = term.astype(bf16)
            if (o, t) in plain:
                tiles = [jnp.concatenate([cv[4 * j + t - 2, q:q + 8] for q in range(8 * (t - 2), 256, 32)], axis=0)
                         for j in range(8)]
            else:
                av = at[len(prepared) & 1].bitcast(u32).at[pl.ds(zero, 7)]
                tiles = [av[t, j] for j in range(8)]
            return jnp.concatenate([
                clk.dot(_as_bf16(jnp.concatenate(tiles[:4], axis=1)), _as_bf16(ww[7 * o + t, c, :256, :]))
                + clk.dot(_as_bf16(jnp.concatenate(tiles[4:], axis=1)), _as_bf16(ww[7 * o + t, c, 256:, :]))
                for c in range(2)], axis=1)

        def emit(i, n, gated_a):
            for q in range(8):
                rr, cc = slice(64 * q + 16 * i, 64 * q + 16 * i + 16), slice(n * 256, (n + 1) * 256)
                b = xv[rr, cc].astype(f32) * jnp.concatenate([yv[2 * n, rr, :], yv[2 * n + 1, rr, :]], axis=1)
                rest = jnp.concatenate([1.0 - gv[rr, :]] * 2, axis=1)
                ov[rr, cc] = (gated_a[16 * q:16 * q + 16] + rest * b).astype(bf16)

        def quadrant_done(q):
            if q in (3, 0):
                start(o_copy(r, q % 2))

        _strassen2(prod, emit, (2, 3, 1, 4, 0, 5, 6), quadrant_done)

    def x_prep(n, _):
        @pl.when((n & 7) == 0)
        def _():
            wait(x_copy(n >> 3))

        rows = [pl.ds(pl.multiple_of((n >> 3) * 512 + (n & 7) * 16 + 128 * i, 16), 16) for i in range(4)]
        out = pl.ds(pl.multiple_of(n * 16, 16), 16)
        gw = gw_s[...].astype(f32)
        logit = [0.0] * 4
        for c in range(2):
            blk = [[x_s[rows[i], k * 256 + c * 128:k * 256 + (c + 1) * 128].astype(f32) for k in range(4)]
                   for i in range(4)]
            scaled = [[b * QSCALE for b in row] for row in blk]
            for o in range(7):
                for t, term in enumerate(_operands2(_LHS, o, lambda i, k: scaled[i][k])):
                    xt[7 * o + t, c, out, :] = term.astype(bf16)
            for i in range(4):
                logit[i] = logit[i] + sum(blk[i][k] * gw[2 * k + c:2 * k + c + 1, :] for k in range(4))
        for i in range(4):
            gate_s[rows[i], :] = logit[i]

    def gate_prep(n, _):
        rows = pl.ds(pl.multiple_of(n * 256, 256), 256)
        gate = jax.nn.sigmoid(jnp.sum(gate_s[rows, :], axis=1, keepdims=True))
        gate_s[rows, :] = jnp.broadcast_to(gate, (256, 128))

    def c_prep(n, _):
        for sub in range(0, 64, 16):
            rows = [pl.ds(pl.multiple_of((n >> 1) * 256 + (n & 1) * 64 + sub + 128 * i, 16), 16) for i in range(2)]
            out = pl.ds(pl.multiple_of(n * 64 + sub, 16), 16)
            for c in range(2):
                quads = [c_s[rows[i], k * 256 + c * 128:k * 256 + (c + 1) * 128].astype(f32)
                         for i in range(2) for k in range(2)]
                for t, term in enumerate(_operands(_LHS, quads)):
                    ct[t, c, out, :] = term.astype(bf16)

    start(small_copies)
    for r in range(4):
        start(x_copy(r))
    start(phase1_copies(0))
    visible = lax.broadcasted_iota(i32, (128, 128), 1) <= lax.broadcasted_iota(i32, (128, 128), 0)
    cap[...] = jnp.where(visible, jnp.inf, -jnp.inf)
    kpad[0:8, :] = jnp.zeros((8, 128), f32)
    wait(small_copies)
    shift, skip = shift_s[...].astype(f32), dd_s[...].astype(f32)
    for n in range(8):
        coef[n, 0:4, :] = shift[:, n * 128:(n + 1) * 128]
        coef[n, 4:5, :] = skip[n:n + 1, :]
    lax.fori_loop(0, 32, x_prep, None)
    lax.fori_loop(0, 8, gate_prep, None)
    wait(phase1_copies(0))
    start(phase1_copies(1))
    lax.fori_loop(0, 8, phase1, None)

    start(q_copy(0) + q_copy(1))
    wait(c_copy + kv_copies(0))
    kv_weight_prep(wk_s.at[0], wkt)
    kv_weight_prep(wv_s.at[0], wvt)
    start(kv_copies(2))
    lax.fori_loop(0, 16, c_prep, None)
    lax.fori_loop(0, NG, phase2, None)

    lax.fori_loop(0, S // 512, phase3, None)
    wait([cp for r in range(S // 512) for half in (1, 0) for cp in o_copy(r, half)])


@jax.jit
def pallas_gated_mix__compressed_kv_cla__ssm_conv_h3__prompt_kernel(
        A_x, A_c_kv, A_w_q, A_w_uk, A_w_uv, A_w_o, B_q, B_k, B_v, B_shift_k, B_ssm_k, B_ssm_D, gate_w):
    del B_q
    hbm = pl.BlockSpec(memory_space=pl.ANY)
    vm = pltpu.VMEM
    out = pl.pallas_call(
        _kernel,
        in_specs=[hbm] * 14,
        out_specs=hbm,
        out_shape=jax.ShapeDtypeStruct((S, M), bf16),
        scratch_shapes=[
            vm((S, M), bf16), vm((49, 2, S // 4, 128), bf16),
            vm((S, DC), bf16), vm((7, 2, S // 2, 128), bf16),
            vm((2, 4, 64, M), bf16), vm((49, 2, 8 * D, 128), bf16),
            vm((H, S, D), bf16), vm((8, S, 128), f32),
            vm((S, M), bf16), vm((S, 128), f32),
            vm((2, S, 128), bf16), vm((2, S, 128), bf16),
            vm((2, 128, S), bf16), vm((2, 2, M, D), u32),
            vm((NC + 1, 2 * C, 128), f32), vm((NC + 1, 2 * C, 128), f32),
            vm((NC + 1, 2 * C, 128), bf16), vm((S + 32, 128), f32),
            vm((2, DC, D), u32), vm((2, DC, D), u32),
            vm((7, DC // 2, D), bf16), vm((7, DC // 2, D), bf16),
            vm((2, 2, S, D), bf16), vm((2, S, D), bf16), vm((2, S, D), bf16),
            vm((128, 128), f32), vm((8, 32, 128), f32),
            vm((2 * C, C), bf16), vm((2 * C, C), bf16),
            [vm((8, M // 4, D), bf16)] * 7,
            [vm((BQ + 32, S), f32)] * NBUF, [vm((BQ, S), bf16)] * NBUF,
            [vm((BQ + 32, 128), f32)] * NBUF, [vm((8, 8, 128, D), bf16)] * 2,
            vm((4, M), bf16), vm((8, 128), bf16), vm((8, 128), bf16),
            pltpu.SemaphoreType.DMA((28,)), pltpu.SemaphoreType.DMA((8,)),
        ],
        compiler_params=pltpu.CompilerParams(vmem_limit_bytes=124 * 2**20),
    )(A_x.reshape(S, M), A_c_kv.reshape(S, DC), A_w_q, A_w_uk, A_w_uv, A_w_o,
      B_k.reshape(S, M), B_v.reshape(S, M), B_ssm_k,
      B_shift_k.T, B_ssm_D.reshape(8, 128), gate_w.reshape(8, 128), _FWD, _INV)
    return out.reshape(1, S, M)
```

```python
import jax
import jax.numpy as jnp
import numpy as np
from jax import lax
from jax.experimental import pallas as pl
from jax.experimental.pallas import tpu as pltpu

S, M, DC, H, D = 2048, 1024, 512, 32, 128
C = 128
NC = S // C
BQ = 256
NB = S // BQ
NG = H // 2
NBUF = 3
f32, bf16, i32, u32 = jnp.float32, jnp.bfloat16, jnp.int32, jnp.uint32
NN = (((1,), (0,)), ((), ()))
NT = (((1,), (1,)), ((), ()))
QSCALE = float(D ** -0.5 * np.log2(np.e))


def _dft_matrices():
    k = np.arange(C)[:, None]
    t = np.arange(C)[None, :]
    ang = 2 * np.pi * (k + 0.25) * t / C
    fwd = np.stack([np.cos(ang).reshape(16, 8, C), np.sin(ang).reshape(16, 8, C)], axis=1).reshape(2 * C, C)
    inv = np.concatenate([fwd.T[:, :C], fwd.T[:, C:]], axis=0) / C
    return fwd.astype(bf16), inv.astype(bf16)


_FWD, _INV = _dft_matrices()

_LHS = (((0, 1), (3, 1)), ((2, 1), (3, 1)), ((0, 1),), ((3, 1),),
        ((0, 1), (1, 1)), ((2, 1), (0, -1)), ((1, 1), (3, -1)))
_RHS = (((0, 1), (3, 1)), ((0, 1),), ((1, 1), (3, -1)), ((2, 1), (0, -1)),
        ((3, 1),), ((0, 1), (1, 1)), ((2, 1), (3, 1)))
_OUT = (((0, 1), (6, 1), (3, 1), (4, -1)), ((2, 1), (4, 1)), ((1, 1), (3, 1)),
        ((0, 1), (5, 1), (1, -1), (2, 1)))
_ORDER = (1, 4, 2, 5, 0, 3, 6)


def _signed_sum(terms, get):
    acc = get(terms[0][0])
    for idx, sign in terms[1:]:
        acc = acc + get(idx) if sign > 0 else acc - get(idx)
    return acc


def _output(n, get, order):
    terms = sorted(_OUT[n], key=lambda term: order.index(term[0]))
    if terms[0][1] < 0:
        terms[:2] = terms[1], terms[0]
    return _signed_sum(terms, get)


def _operands(table, quads):
    return [_signed_sum(terms, lambda n: quads[n]) for terms in table]


def _operands2(table, outer, block):
    return _operands(table, [
        _signed_sum(table[outer], lambda n: block(2 * (n // 2) + i, 2 * (n % 2) + j))
        for i in range(2) for j in range(2)])


def _finished(order):
    last = [max(order.index(t) for t, _ in terms) for terms in _OUT]
    return [[n for n in range(4) if last[n] == pos] for pos in range(7)]


def _strassen(prod, order):
    m = {t: prod(t) for t in order}
    return [_output(n, lambda t: m[t], order) for n in range(4)]


def _strassen2(prod, emit, order, quadrant_done=lambda n: None):
    m = {}
    for o, done in zip(order, _finished(order)):
        m[o] = _strassen(lambda t: prod(o, t), order)
        for q in done:
            for n in sum(_finished(order), []):
                emit(2 * (q // 2) + n // 2, 2 * (q % 2) + n % 2, _output(q, lambda t: m[t][n], order))
            quadrant_done(q)


class _Clock:
    def __init__(self, zero=None):
        self.busy = [0, 0, 0, 0]
        self.marks = []
        self.jobs = []
        if zero is not None:
            self.zero = jnp.full((8, 128), zero, i32)

    @property
    def t(self):
        return min(self.busy)

    def advance(self, rows, tiles):
        for _ in range(tiles):
            u = self.busy.index(min(self.busy))
            begin = self.busy[u]
            self.busy[u] += rows
        return begin

    def run_due(self, when):
        ready = [j for j in self.jobs if j[0] < when]
        self.jobs = [j for j in self.jobs if j[0] >= when]
        out = [(t, job()) for t, job in ready]
        return [o for o in out if o[1] is not None]

    def dot(self, a, b, dims=NN):
        rows, first = a.shape[0], self.t
        ready = self.run_due(first + rows)
        if ready:
            words = pltpu.bitcast(a[:, :128], i32)
            parts = [words[r:r + 8] for r in range(0, rows // 2, 8)]
            for t, val in ready:
                n = int(max(t - first, 0)) // 16
                parts[n] = parts[n] | (pltpu.bitcast(val, i32) & self.zero)
            head = pltpu.bitcast(jnp.concatenate(parts, axis=0), bf16)
            a = head if a.shape[1] == 128 else jnp.concatenate([head, a[:, 128:]], axis=1)
        out = lax.dot_general(a, b, dims, preferred_element_type=f32)
        begin = self.advance(rows, a.shape[1] // 128)
        self.marks += [(begin + r + 8, out, r) for r in range(0, rows, 8)]
        return out

    def after(self, when):
        _, val, r = max((m for m in self.marks if m[0] <= max(when, 8)), key=lambda m: m[0])
        nothing = pltpu.bitcast(val[r:r + 8, :], i32) & self.zero

        def hold(x):
            words = pltpu.bitcast(x, i32)
            return pltpu.bitcast(words | jnp.concatenate([nothing] * (words.shape[0] // 8), axis=0), x.dtype)
        return hold


PACE, MINPACE, WINDOW = 5.45, 3.9, 780


def _attention_plan():
    steps = [("k", 0), ("k", 1)]
    for u in range(2 * NB + NBUF - 1):
        if u < 2 * NB:
            steps.append(("qk", u))
        if u % 2 == 0 and 1 < u // 2 + 1 < NB:
            steps.append(("k", u // 2 + 1))
        if u % 2 == 1 and u < 2 * NB:
            steps.append(("v", u // 2))
        if u >= NBUF - 1:
            steps.append(("pv", u - NBUF + 1))
    clk, scored, needed = _Clock(), {}, {}
    for kind, u in steps:
        if kind == "qk":
            clk.advance(BQ, u // 2 * 2 + 1)
            clk.advance(128, 1)
            scored[u] = max(clk.busy)
        elif kind == "pv":
            for half in range(2):
                needed[u, half] = clk.t
                clk.advance(128, u // 2 * 2 + 1 + half)
        else:
            clk.advance(128, 14)
    groups = [(u, r) for u in range(2 * NB) for r in range(0, BQ, 8)]
    work = [u // 2 * 2 + 1 + r // 128 for u, r in groups]
    times, t = [], 0
    for (u, r), w in zip(groups, work):
        t = max(t, scored[u])
        times.append(t)
        t += PACE * w
    t = clk.t
    for n in reversed(range(len(groups))):
        u, r = groups[n]
        t = times[n] = min(times[n], needed[u, r // 128] - WINDOW, t - MINPACE * work[n])
    return steps, dict(zip(groups, times))


def _on_first_tile(fn, x):
    return fn(x) if x.shape[1] == 128 else jnp.concatenate([fn(x[:, :128]), x[:, 128:]], axis=1)


def _as_bf16(words):
    return pltpu.bitcast(words, bf16)


def _head(words, e):
    return pltpu.bitcast(words & np.uint32(0xFFFF0000) if e else words << 16, f32)


def _kernel(x_hbm, c_hbm, wq_hbm, wk_hbm, wv_hbm, wo_hbm, bk_hbm, bv_hbm, hk_hbm,
            shift_hbm, dd_hbm, gw_hbm, fwd_hbm, inv_hbm, o_hbm,
            x_s, xt, c_s, ct, wo_s, wot, ctx, yb, o_s, gate_s,
            bk_s, bv_s, hk_s, wq_s, xsp, hsp, qsp, kpad,
            wk_s, wv_s, wkt, wvt, q_s, k_s, v_s, cap, coef, fwd_s, inv_s,
            wqt, sb, pb, lb, at, shift_s, dd_s, gw_s, sem, osem):
    copy = pltpu.make_async_copy

    def start(copies):
        for cp in copies:
            cp.start()

    def wait(copies):
        for cp in copies:
            cp.wait()

    def x_copy(r):
        rows = pl.ds(pl.multiple_of(r * 512, 512), 512)
        return [copy(x_hbm.at[rows], x_s.at[rows], sem.at[r])]

    c_copy = [copy(c_hbm, c_s, sem.at[4])]
    small_copies = [copy(a, b, sem.at[5 + n]) for n, (a, b) in enumerate(
        ((shift_hbm, shift_s), (dd_hbm, dd_s), (gw_hbm, gw_s), (fwd_hbm, fwd_s), (inv_hbm, inv_s)))]

    def phase1_copies(n):
        cols = pl.ds(pl.multiple_of(n * 128, 128), 128)
        s = n & 1
        return [copy(hk_hbm.at[cols, :], hk_s.at[s], sem.at[10 + s]),
                copy(bk_hbm.at[:, cols], bk_s.at[s], sem.at[12 + s]),
                copy(bv_hbm.at[:, cols], bv_s.at[s], sem.at[14 + s]),
                copy(wq_hbm.bitcast(u32).at[:, 2 * n, :], wq_s.at[s, 0], sem.at[16 + s]),
                copy(wq_hbm.bitcast(u32).at[:, 2 * n + 1, :], wq_s.at[s, 1], sem.at[18 + s])]

    def kv_copies(g):
        return [copy(wk_hbm.bitcast(u32).at[:, g, :], wk_s.at[g & 1], sem.at[20 + (g & 1)]),
                copy(wv_hbm.bitcast(u32).at[:, g, :], wv_s.at[g & 1], sem.at[22 + (g & 1)])]

    def wo_copy(g):
        src = wo_hbm.at[pl.ds((g >> 1) * 4, 4), pl.ds(pl.multiple_of((g & 1) * 64, 64), 64), :]
        return [copy(src, wo_s.at[g & 1], sem.at[24 + (g & 1)])]

    def q_copy(g):
        return [copy(ctx.at[pl.ds(2 * g, 2)], q_s.at[g & 1], sem.at[26 + (g & 1)])]

    def o_copy(r, half):
        rows, cols = pl.ds(pl.multiple_of(r * 512, 512), 512), pl.ds(half * 512, 512)
        return [copy(o_s.at[rows, cols], o_hbm.at[rows, cols], osem.at[2 * r + half])]

    def lhs_operand(ref, t, blk):
        words = ref.bitcast(u32)
        return _as_bf16(jnp.concatenate([words[t, c, blk * 64:(blk + 1) * 64, :] for c in range(2)], axis=1))

    def kv_weight_prep(raw, dst, hold_at=lambda frac: (lambda x: x)):
        for r in range(0, DC // 2, 16):
            hold = hold_at(r / (DC // 2))
            words = [hold(raw[a:a + 16, :]) for a in (r, DC // 2 + r)]
            for t, term in enumerate(_operands(_RHS, [_head(w, e) for w in words for e in range(2)])):
                dst[t, r:r + 16, :] = term.astype(bf16)


    def phase1(it, _):
        @pl.when(it > 0)
        def _():
            wait(phase1_copies(it))

        zero = it >> 6
        clk = _Clock(zero)
        s = it & 1
        fwd = _as_bf16(fwd_s.bitcast(u32)[...])
        kpad[8:8 + S, :] = bk_s[s].astype(f32)
        taps = [coef[it, j:j + 1, :] for j in range(4)]
        for m in range(NC + 2):
            if m < NC:
                hsp[m] = clk.dot(fwd, hk_s[s, :, m * C:(m + 1) * C], NT)
            j = m - 2
            if j >= 0:
                ks = sum(kpad[8 - t + j * C:8 - t + (j + 1) * C, :] * taps[t] for t in range(4))
                kv = (ks * bv_s[s, j * C:(j + 1) * C, :].astype(f32)).astype(bf16)
                xsp[j] = clk.dot(fwd, kv)

        prepared = []

        def q_prod(blk, o, t):
            if o not in prepared:
                prepared.append(o)
                for r in range(0, M // 4, 16):
                    hold = clk.after(clk.t - 260 - 450 * (1 - r / (M // 4)))
                    terms = _operands2(_RHS, o, lambda k, hd: _head(
                        hold(wq_s[s, hd // 2, k * (M // 4) + r:k * (M // 4) + r + 16, :]), hd % 2))
                    for n, term in enumerate(terms):
                        wqt[o][n, r:r + 16, :] = term.astype(bf16)
            return clk.dot(lhs_operand(xt, 7 * o + t, blk), _as_bf16(wqt[o].bitcast(u32).at[pl.ds(zero, 7)][t]))

        for blk in range(S // 512):
            def q_emit(i, hd, val):
                ctx[4 * it + hd, blk * 512 + i * 128:blk * 512 + (i + 1) * 128, :] = val.astype(bf16)
            _strassen2(lambda o, t: q_prod(blk, o, t), q_emit, _ORDER)

        hsp[NC, :8, :] = clk.after(4400)(cap[:8, :])
        skip = coef[it, 4:5, :]
        hv, xv = hsp.at[pl.ds(zero, NC)], xsp.at[pl.ds(zero, NC)]
        for f in range(16):
            re, im = slice(16 * f, 16 * f + 8), slice(16 * f + 8, 16 * f + 16)
            hr = [hv[m, re, :] for m in range(NC)]
            hi = [hv[m, im, :] for m in range(NC)]
            hr[0] = hr[0] + skip
            xr = [xv[j, re, :] for j in range(NC)]
            xi = [xv[j, im, :] for j in range(NC)]
            pr = pi = None
            for i in range(NC):
                ar = ai = None
                for j in range(i + 1):
                    tr = hr[i - j] * xr[j] - hi[i - j] * xi[j]
                    ti = hr[i - j] * xi[j] + hi[i - j] * xr[j]
                    ar = tr if ar is None else ar + tr
                    ai = ti if ai is None else ai + ti
                qr, qi = (ar, ai) if pr is None else (ar + pi, ai - pr)
                pr, pi = ar, ai
                qsp[i, 16 * f:16 * f + 16, :] = jnp.concatenate([qr, qi], axis=0).astype(bf16)
        iw = inv_s.bitcast(u32)
        inv = _as_bf16(jnp.concatenate([iw[:C // 2, :], iw[C // 2:, :]], axis=1))
        qv = qsp.bitcast(u32).at[pl.ds(zero, NC)]
        for i in range(NC):
            yb[it, i * C:(i + 1) * C, :] = jnp.dot(inv, _as_bf16(qv[i]), preferred_element_type=f32)

        @pl.when(it < 6)
        def _():
            start(phase1_copies(it + 2))

        @pl.when(it == 6)
        def _():
            start(c_copy + wo_copy(0) + wo_copy(1) + kv_copies(0) + kv_copies(1))

    def phase2(g, _):
        @pl.when(g < NG - 1)
        def _():
            wait(kv_copies(g + 1))

        wait(wo_copy(g) + q_copy(g))
        zero = g >> 6
        first, second = (pl.ds(pl.multiple_of((g >> n) * 32, 32), BQ) for n in (7, 6))
        clk = _Clock(zero)
        qw = q_s.bitcast(u32).at[g & 1]
        steps, begin = _attention_plan()

        def up_project(i, wt, dst):
            out = _strassen(lambda t: clk.dot(lhs_operand(ct, t, i), _as_bf16(wt.bitcast(u32)[t])), _ORDER)
            for n, val in enumerate(out):
                r = i * BQ + 128 * (n // 2)
                dst[n % 2, r:r + 128, :] = val.astype(bf16)

        def scores(u):
            i, e = divmod(u, 2)
            for j in range(2 * i + 2):
                r0 = 128 if j == 2 * i + 1 else 0
                s = clk.dot(_as_bf16(qw[e, (i * BQ + r0) // 2:(i + 1) * BQ // 2, :]),
                            k_s[e, j * 128:(j + 1) * 128, :], NT)
                if j == 2 * i:
                    s = jnp.concatenate([jnp.minimum(s[:128], cap[...]), s[128:]], axis=0)
                if j == 2 * i + 1:
                    s = jnp.minimum(s, cap[...])
                sb[u % NBUF][r0:BQ, j * 128:(j + 1) * 128] = s
            for r0 in range(0, BQ, 8):
                clk.jobs.append((begin[u, r0] + WINDOW, lambda r0=r0: softmax(u, r0)))

        def softmax(u, r0):
            i = u // 2
            r = slice(r0, r0 + 8)
            keys = (2 * i + 1 + r0 // 128) * 128
            top = jnp.max(_on_first_tile(clk.after(begin[u, r0]), sb[u % NBUF].at[first][r, :keys]),
                          axis=1, keepdims=True)
            p = jnp.exp2(sb[u % NBUF].at[second][r, :keys] - top)
            norm = pltpu.reciprocal(jnp.sum(p, axis=1, keepdims=True), full_range=False)
            norm = jnp.broadcast_to(norm, (8, 128))
            lb[u % NBUF][r, :] = norm * gate_s[i * BQ + r0:i * BQ + r0 + 8, :]
            short = u < 8
            if short:
                p = _on_first_tile(lambda x: jnp.maximum(x, -norm), p)
            pb[u % NBUF][r, :keys] = p.astype(bf16)
            return None if short else norm

        def context(u):
            i, e = divmod(u, 2)
            for r0 in range(0, BQ, 128):
                clk.run_due(clk.t + 1)
                acc = None
                for j in range(2 * i + 1 + r0 // 128):
                    part = clk.dot(pb[u % NBUF][r0:r0 + 128, j * 128:(j + 1) * 128], v_s[e, j * 128:(j + 1) * 128, :])
                    acc = part if acc is None else acc + part
                row = i * BQ + r0
                ctx[2 * g + e, row:row + 128, :] = (acc * lb[u % NBUF].at[second][r0:r0 + 128, :]).astype(bf16)
                stored = ctx.bitcast(u32)[2 * g + e + zero, row // 2:row // 2 + 8, :]
                clk.jobs.append((max(clk.busy) + 400, lambda stored=stored: stored))

        for kind, u in steps:
            if kind == "k":
                up_project(u, wkt, k_s)
                k_done = clk.t
            elif kind == "v":
                up_project(u, wvt, v_s)
            elif kind == "qk":
                scores(u)
            else:
                context(u)

        kv_weight_prep(wk_s.at[(g + 1) & 1], wkt, lambda frac: clk.after(k_done + frac * 2000))
        kv_weight_prep(wv_s.at[(g + 1) & 1], wvt, lambda frac: clk.after(clk.t - 900 + frac * 600))
        wsrc = wo_s.at[g & 1]
        for r in range(0, 64, 16):
            out = pl.ds(pl.multiple_of(g * 64 + r, 16), 16)
            for c in range(2):
                for o in range(7):
                    hold = clk.after(((r // 8 + c) * 7 + o) * 24)
                    terms = _operands2(_RHS, o, lambda k, n: hold(
                        wsrc[k, r:r + 16, n * 256 + c * 128:n * 256 + (c + 1) * 128]).astype(f32))
                    for t, term in enumerate(terms):
                        wot[7 * o + t, c, out, :] = term.astype(bf16)

        @pl.when(g < NG - 3)
        def _():
            start(kv_copies(g + 3))

        @pl.when(g < NG - 2)
        def _():
            start(wo_copy(g + 2) + q_copy(g + 2))

    def phase3(r, _):
        zero = r >> 6
        clk = _Clock(zero)
        cv = ctx.bitcast(u32).at[:, pl.ds(pl.multiple_of(r * 256, 256), 256)]
        ww = wot.bitcast(u32)
        rows = pl.ds(pl.multiple_of(r * 512, 512), 512)
        yv, xv, gv, ov = yb.at[:, rows], x_s.at[rows], gate_s.at[rows], o_s.at[rows]
        plain = ((2, 2), (2, 3))
        prepared = []

        def prod(o, t):
            if (o, t) not in plain and o not in prepared:
                prepared.append(o)
                end = clk.t - 260
                for j in range(8):
                    for q in range(8):
                        hold = clk.after(end - min(end, 3000) * (1 - (j * 8 + q) / 64))
                        terms = _operands2(_LHS, o, lambda i, k: _as_bf16(
                            hold(cv[4 * j + k, 32 * q + 8 * i:32 * q + 8 * i + 8])).astype(f32))
                        for n, term in enumerate(terms):
                            if (o, n) not in plain:
                                at[len(prepared) & 1][n, j, 16 * q:16 * q + 16] = term.astype(bf16)
            if (o, t) in plain:
                tiles = [jnp.concatenate([cv[4 * j + t - 2, q:q + 8] for q in range(8 * (t - 2), 256, 32)], axis=0)
                         for j in range(8)]
            else:
                av = at[len(prepared) & 1].bitcast(u32).at[pl.ds(zero, 7)]
                tiles = [av[t, j] for j in range(8)]
            return jnp.concatenate([
                clk.dot(_as_bf16(jnp.concatenate(tiles[:4], axis=1)), _as_bf16(ww[7 * o + t, c, :256, :]))
                + clk.dot(_as_bf16(jnp.concatenate(tiles[4:], axis=1)), _as_bf16(ww[7 * o + t, c, 256:, :]))
                for c in range(2)], axis=1)

        def emit(i, n, gated_a):
            for q in range(8):
                rr, cc = slice(64 * q + 16 * i, 64 * q + 16 * i + 16), slice(n * 256, (n + 1) * 256)
                b = xv[rr, cc].astype(f32) * jnp.concatenate([yv[2 * n, rr, :], yv[2 * n + 1, rr, :]], axis=1)
                rest = jnp.concatenate([1.0 - gv[rr, :]] * 2, axis=1)
                ov[rr, cc] = (gated_a[16 * q:16 * q + 16] + rest * b).astype(bf16)

        def quadrant_done(q):
            if q in (3, 0):
                start(o_copy(r, q % 2))

        _strassen2(prod, emit, (2, 3, 1, 4, 0, 5, 6), quadrant_done)

    def x_prep(n, _):
        @pl.when((n & 7) == 0)
        def _():
            wait(x_copy(n >> 3))

        rows = [pl.ds(pl.multiple_of((n >> 3) * 512 + (n & 7) * 16 + 128 * i, 16), 16) for i in range(4)]
        out = pl.ds(pl.multiple_of(n * 16, 16), 16)
        gw = gw_s[...].astype(f32)
        logit = [0.0] * 4
        for c in range(2):
            blk = [[x_s[rows[i], k * 256 + c * 128:k * 256 + (c + 1) * 128].astype(f32) for k in range(4)]
                   for i in range(4)]
            scaled = [[b * QSCALE for b in row] for row in blk]
            for o in range(7):
                for t, term in enumerate(_operands2(_LHS, o, lambda i, k: scaled[i][k])):
                    xt[7 * o + t, c, out, :] = term.astype(bf16)
            for i in range(4):
                logit[i] = logit[i] + sum(blk[i][k] * gw[2 * k + c:2 * k + c + 1, :] for k in range(4))
        for i in range(4):
            gate_s[rows[i], :] = logit[i]

    def gate_prep(n, _):
        rows = pl.ds(pl.multiple_of(n * 256, 256), 256)
        gate = jax.nn.sigmoid(jnp.sum(gate_s[rows, :], axis=1, keepdims=True))
        gate_s[rows, :] = jnp.broadcast_to(gate, (256, 128))

    def c_prep(n, _):
        for sub in range(0, 64, 16):
            rows = [pl.ds(pl.multiple_of((n >> 1) * 256 + (n & 1) * 64 + sub + 128 * i, 16), 16) for i in range(2)]
            out = pl.ds(pl.multiple_of(n * 64 + sub, 16), 16)
            for c in range(2):
                quads = [c_s[rows[i], k * 256 + c * 128:k * 256 + (c + 1) * 128].astype(f32)
                         for i in range(2) for k in range(2)]
                for t, term in enumerate(_operands(_LHS, quads)):
                    ct[t, c, out, :] = term.astype(bf16)

    start(small_copies)
    for r in range(4):
        start(x_copy(r))
    start(phase1_copies(0))
    visible = lax.broadcasted_iota(i32, (128, 128), 1) <= lax.broadcasted_iota(i32, (128, 128), 0)
    cap[...] = jnp.where(visible, jnp.inf, -jnp.inf)
    kpad[0:8, :] = jnp.zeros((8, 128), f32)
    wait(small_copies)
    shift, skip = shift_s[...].astype(f32), dd_s[...].astype(f32)
    for n in range(8):
        coef[n, 0:4, :] = shift[:, n * 128:(n + 1) * 128]
        coef[n, 4:5, :] = skip[n:n + 1, :]
    lax.fori_loop(0, 32, x_prep, None)
    lax.fori_loop(0, 8, gate_prep, None)
    wait(phase1_copies(0))
    start(phase1_copies(1))
    lax.fori_loop(0, 8, phase1, None)

    start(q_copy(0) + q_copy(1))
    wait(c_copy + kv_copies(0))
    kv_weight_prep(wk_s.at[0], wkt)
    kv_weight_prep(wv_s.at[0], wvt)
    start(kv_copies(2))
    lax.fori_loop(0, 16, c_prep, None)
    lax.fori_loop(0, NG, phase2, None)

    lax.fori_loop(0, S // 512, phase3, None)
    wait([cp for r in range(S // 512) for half in (1, 0) for cp in o_copy(r, half)])


@jax.jit
def pallas_gated_mix__compressed_kv_cla__ssm_conv_h3__prompt_kernel(
        A_x, A_c_kv, A_w_q, A_w_uk, A_w_uv, A_w_o, B_q, B_k, B_v, B_shift_k, B_ssm_k, B_ssm_D, gate_w):
    del B_q
    hbm = pl.BlockSpec(memory_space=pl.ANY)
    vm = pltpu.VMEM
    out = pl.pallas_call(
        _kernel,
        in_specs=[hbm] * 14,
        out_specs=hbm,
        out_shape=jax.ShapeDtypeStruct((S, M), bf16),
        scratch_shapes=[
            vm((S, M), bf16), vm((49, 2, S // 4, 128), bf16),
            vm((S, DC), bf16), vm((7, 2, S // 2, 128), bf16),
            vm((2, 4, 64, M), bf16), vm((49, 2, 8 * D, 128), bf16),
            vm((H, S, D), bf16), vm((8, S, 128), f32),
            vm((S, M), bf16), vm((S, 128), f32),
            vm((2, S, 128), bf16), vm((2, S, 128), bf16),
            vm((2, 128, S), bf16), vm((2, 2, M, D), u32),
            vm((NC + 1, 2 * C, 128), f32), vm((NC + 1, 2 * C, 128), f32),
            vm((NC + 1, 2 * C, 128), bf16), vm((S + 32, 128), f32),
            vm((2, DC, D), u32), vm((2, DC, D), u32),
            vm((7, DC // 2, D), bf16), vm((7, DC // 2, D), bf16),
            vm((2, 2, S, D), bf16), vm((2, S, D), bf16), vm((2, S, D), bf16),
            vm((128, 128), f32), vm((8, 32, 128), f32),
            vm((2 * C, C), bf16), vm((2 * C, C), bf16),
            [vm((8, M // 4, D), bf16)] * 7,
            [vm((BQ + 32, S), f32)] * NBUF, [vm((BQ, S), bf16)] * NBUF,
            [vm((BQ + 32, 128), f32)] * NBUF, [vm((8, 8, 128, D), bf16)] * 2,
            vm((4, M), bf16), vm((8, 128), bf16), vm((8, 128), bf16),
            pltpu.SemaphoreType.DMA((28,)), pltpu.SemaphoreType.DMA((8,)),
        ],
        compiler_params=pltpu.CompilerParams(vmem_limit_bytes=124 * 2**20),
    )(A_x.reshape(S, M), A_c_kv.reshape(S, DC), A_w_q, A_w_uk, A_w_uv, A_w_o,
      B_k.reshape(S, M), B_v.reshape(S, M), B_ssm_k,
      B_shift_k.T, B_ssm_D.reshape(8, 128), gate_w.reshape(8, 128), _FWD, _INV)
    return out.reshape(1, S, M)
```
